```python
import os as _os
_os.environ.setdefault("JAX_PLATFORMS", "cpu")
import jax
import jax.numpy as jnp

def _softmax(x, axis=-1):
    return jax.nn.softmax(x, axis=axis)
def _gelu(x):
    return jax.nn.gelu(x, approximate=True)
def _silu(x):
    return jax.nn.silu(x)
def _sigmoid(x):
    return jax.nn.sigmoid(x)
def _layernorm(x, axis=-1, eps=1e-5):
    m = jnp.mean(x, axis=axis, keepdims=True)
    v = jnp.var(x, axis=axis, keepdims=True)
    return (x - m) / jnp.sqrt(v + eps)
def _scatter_add(tgt, idx, src, axis=0):
    return tgt.at[idx].add(src)
def _segment_sum(src, seg, n):
    return jax.ops.segment_sum(src, seg, n)
class _Rng:
    def __init__(self, key):
        self._k = key
    def _next(self):
        self._k, sub = jax.random.split(self._k)
        return sub
    def normal(self, shape):
        return jax.random.normal(self._next(), shape, dtype=jnp.bfloat16)
    def randint(self, lo, hi, shape):
        return jax.random.randint(self._next(), shape, lo, hi, dtype=jnp.int32)
    def uniform(self, shape, lo=0.0, hi=1.0):
        return jax.random.uniform(self._next(), shape, jnp.bfloat16, lo, hi)
    def permutation(self, n):
        return jax.random.permutation(self._next(), n)


kernel_name = 'sequential_preLN__mha_block__moe_arch_mod__prompt'

def setup_inputs():
    _rng = _Rng(jax.random.key(int.from_bytes(__import__("os").urandom(4), "little")))
    _w = (lambda a: (lambda t: t.astype(jnp.bfloat16) if jnp.issubdtype(t.dtype, jnp.floating) else t)(jnp.asarray(a)))
    def _A_setup():
        B, S, D, H = 1, 2048, 640, 32
        return {
            "x": _w((lambda *s: _rng.normal(s) * 0.05)(B, S, D)),
            "wqkv": _w((lambda *s: _rng.normal(s) * 0.05)(D, 3 * D)),
            "wo": _w((lambda *s: _rng.normal(s) * 0.05)(D, D)),
        }
    _A_in = _A_setup()

    def _B_setup():
        B, S, D, F, C = 1, 2048, 640, 1536, 1
        return {
            "x": _w((lambda *s: _rng.normal(s) * 0.05)(B, S, D)),
            "w_r": _w((lambda *s: _rng.normal(s) * 0.05)(D)),
            "w_gate": _w((lambda *s: _rng.normal(s) * 0.05)(D, F)),
            "w_up": _w((lambda *s: _rng.normal(s) * 0.05)(D, F)),
            "w_down": _w((lambda *s: _rng.normal(s) * 0.05)(F, D)),
        }
    _B_in = _B_setup()

    return {
        "A_x": _A_in["x"],
        "A_wqkv": _A_in["wqkv"],
        "A_wo": _A_in["wo"],
        "B_x": _B_in["x"],
        "B_w_r": _B_in["w_r"],
        "B_w_gate": _B_in["w_gate"],
        "B_w_up": _B_in["w_up"],
        "B_w_down": _B_in["w_down"],
    }

def reference(A_x, A_wqkv, A_wo, B_x, B_w_r, B_w_gate, B_w_up, B_w_down):
    def _A_ref(x, wqkv, wo):
        B, S, D = x.shape
        H = 32
        Dh = D // H
        qkv = (lambda x, *d: x.transpose(*d))((x @ wqkv).reshape(B, S, 3, H, Dh), 2, 0, 3, 1, 4)
        q, k, v = qkv[0], qkv[1], qkv[2]
        scores = jnp.einsum("bhqd,bhkd->bhqk", q, k) * (Dh ** -0.5)
        p = _softmax(scores, axis=-1)
        o = jnp.einsum("bhqk,bhkd->bhqd", p, v)
        return (lambda x, *d: x.transpose(*d))(o, 0, 2, 1, 3).reshape(B, S, D) @ wo

    def _B_ref(x, w_r, w_gate, w_up, w_down):
        B, S, D = x.shape
        C = 1
        r = x @ w_r
        idx = jnp.argsort(-r, axis=-1)[:, :C]
        idx_e = jnp.repeat(idx.reshape(B, C, 1), D, axis=2)
        x_sel = jnp.take_along_axis(x, idx_e, axis=1)
        g = _silu(x_sel @ w_gate)
        u = x_sel @ w_up
        y = (g * u) @ w_down
        r_sel = _sigmoid(jnp.take_along_axis(r, idx, axis=1))
        y = y * r_sel.reshape(B, C, 1)
        b_off = (jnp.arange(B) * S).reshape(B, 1)
        flat_idx = (idx + b_off).reshape(B * C)
        zero = (x * 0.0).reshape(B * S, D)
        upd = _scatter_add(zero, flat_idx, y.reshape(B * C, D), axis=0)
        return x + upd.reshape(B, S, D)

    x = A_x
    h = x + _A_ref(_layernorm(x, axis=-1), A_wqkv, A_wo)
    h2 = h + _B_ref(_layernorm(h, axis=-1), B_w_r, B_w_gate, B_w_up, B_w_down)
    return h2
```

```python
import functools
import math

import jax
import jax.numpy as jnp
import numpy as np
from jax import lax
from jax.experimental import pallas as pl
from jax.experimental.pallas import tpu as pltpu

S = 2048
D = 640
H = 32
DH = 20
F = 1536
QB = 512
KC = 128
NQB = S // QB
NKC = S // KC
TC = 256
NTC = S // TC
EPS = 1e-5
LOG2E = 1.4426950408889634
QSCALE = float(DH ** -0.5 * LOG2E)
NEG = -1e30
SPB = 4

BF16 = jnp.bfloat16
F32 = jnp.float32


def _dot(a, b):
    return jnp.dot(a, b, preferred_element_type=F32)


def _dot_nt(a, b):
    return lax.dot_general(a, b, (((1,), (1,)), ((), ())), preferred_element_type=F32)


def _layernorm_rows(x):
    mu = jnp.mean(x, axis=-1, keepdims=True)
    xc = x - mu
    var = jnp.mean(xc * xc, axis=-1, keepdims=True)
    return xc * lax.rsqrt(var + EPS)


def _kernel(x_ref, wqkv_ref, wr_ref, wo_hbm, wg_hbm, wu_hbm, wd_hbm,
            out_ref,
            wo_ref, wg_ref, wu_ref, wd_ref, sems,
            wqvt_ref, kp_ref, qt_ref, vt_ref, s_ref, ot_ref, hn_ref, r_ref):
    copies = [
        pltpu.make_async_copy(wo_hbm, wo_ref, sems.at[0]),
        pltpu.make_async_copy(wg_hbm, wg_ref, sems.at[1]),
        pltpu.make_async_copy(wu_hbm, wu_ref, sems.at[2]),
        pltpu.make_async_copy(wd_hbm, wd_ref, sems.at[3]),
    ]
    for c in copies:
        c.start()

    with jax.named_scope("wT"):
        wqvt_ref[0:D, :] = wqkv_ref[:, 0:D].T
        wqvt_ref[D:2 * D, :] = wqkv_ref[:, 2 * D:3 * D].T

    lane32 = lax.broadcasted_iota(jnp.int32, (TC, 32), 1)

    def proj(c, carry):
        rows = pl.ds(pl.multiple_of(c * TC, TC), TC)
        xn = _layernorm_rows(x_ref[rows, :].astype(F32)).astype(BF16)
        k = _dot(xn, wqkv_ref[:, D:2 * D])
        for h in range(H):
            o = 16 * ((DH * h) // 16)
            lo = DH * h - o
            kw = k[:, o:o + 32]
            kw = jnp.where((lane32 >= lo) & (lane32 < lo + DH), kw, 0.0)
            kp_ref[h, rows, :] = kw.astype(BF16)
        qv = _dot_nt(wqvt_ref[...], xn)
        j = c // (QB // TC)
        lanes = pl.ds(pl.multiple_of((c % (QB // TC)) * TC, TC), TC)
        qt_ref[j, :, lanes] = (qv[0:D, :] * QSCALE).astype(BF16)
        for u in range(TC // KC):
            vt_ref[c * (TC // KC) + u, :, :] = qv[D:2 * D, u * KC:(u + 1) * KC]
        return carry

    with jax.named_scope("proj"):
        lax.fori_loop(0, NTC, proj, 0)

    def chunk_rows(kc):
        if isinstance(kc, int):
            return pl.ds(kc * KC, KC)
        return pl.ds(pl.multiple_of(kc * KC, KC), KC)

    def qk(j, h, kc):
        o = pl.multiple_of(((DH * h) // 16) * 16, 16)
        k = kp_ref[h, chunk_rows(kc), :]
        qt = qt_ref[j, pl.ds(o, 32), :]
        return _dot(k, qt)

    def upd_max(m, s):
        return jnp.maximum(m, jnp.max(s.reshape(KC // 8, 8, QB), axis=0))

    def finish_max(m):
        return jnp.broadcast_to(jnp.max(m, axis=0, keepdims=True), (8, QB))

    row24 = lax.broadcasted_iota(jnp.int32, (24, KC), 0)
    row8 = lax.broadcasted_iota(jnp.int32, (8, QB), 0)

    def step(j, h, par, m_cur, nxt):
        ones_row = 20 if par == 0 else 0
        ov = pl.multiple_of(((DH * h) // 8) * 8, 8)
        m_new = jnp.full((8, QB), NEG, F32)
        acc = jnp.zeros((24, QB), F32)
        for kc in range(NKC):
            s_old = s_ref[chunk_rows(kc), :]
            if nxt is not None:
                s_new = qk(nxt[0], nxt[1], kc)
            p = jnp.exp2((s_old.reshape(KC // 8, 8, QB) - m_cur[None]).reshape(KC, QB)).astype(BF16)
            vt = vt_ref[kc, pl.ds(ov, 24), :]
            vt = jnp.where(row24 == ones_row, 1.0, vt)
            acc = acc + _dot(vt, p)
            if nxt is not None:
                s_ref[chunk_rows(kc), :] = s_new
                m_new = upd_max(m_new, s_new)
        inv_l = 1.0 / acc[ones_row:ones_row + 1, :]
        o_n = acc * inv_l
        if par == 0:
            ot_ref[j, pl.ds(ov, 24), :] = o_n
        else:
            first = ot_ref[j, pl.ds(ov, 8), :]
            ot_ref[j, pl.ds(ov, 8), :] = jnp.where(row8 < 4, first, o_n[0:8, :])
            ot_ref[j, pl.ds(ov + 8, 16), :] = o_n[8:24, :]
        return finish_max(m_new)

    def prologue(kc, m):
        s = qk(0, 0, kc)
        s_ref[chunk_rows(kc), :] = s
        return upd_max(m, s)

    with jax.named_scope("attn_pro"):
        m0 = finish_max(lax.fori_loop(0, NKC, prologue, jnp.full((8, QB), NEG, F32)))

    NB = NQB * H // SPB

    def body(b, m, last=False):
        t0 = b * SPB
        j = t0 // H
        h0 = t0 % H
        for u in range(SPB):
            if u < SPB - 1:
                nxt = (j, h0 + u + 1)
            elif last:
                nxt = None
            else:
                t1 = t0 + SPB
                nxt = (t1 // H, t1 % H)
            m = step(j, h0 + u, u % 2, m, nxt)
        return m

    with jax.named_scope("attn"):
        m = lax.fori_loop(0, NB - 1, body, m0)
        body(NB - 1, m, last=True)

    copies[0].wait()
    wr = wr_ref[...].astype(F32)

    def post(c, carry):
        rows = pl.ds(pl.multiple_of(c * TC, TC), TC)
        j = c // (QB // TC)
        lanes = pl.ds(pl.multiple_of((c % (QB // TC)) * TC, TC), TC)
        o = ot_ref[j, :, lanes].T.astype(BF16)
        attn = _dot(o, wo_ref[...])
        hh = x_ref[rows, :].astype(F32) + attn
        hn = _layernorm_rows(hh)
        out_ref[rows, :] = (hh + hn).astype(BF16)
        hnb = hn.astype(BF16)
        hn_ref[rows, :] = hnb
        r_ref[rows, :] = jnp.sum(hnb.astype(F32) * wr, axis=-1, keepdims=True)
        return carry

    with jax.named_scope("post"):
        lax.fori_loop(0, NTC, post, 0)

    with jax.named_scope("ffn"):
        r = r_ref[...]
        rmax = jnp.max(r)
        tok = lax.broadcasted_iota(jnp.int32, (S, 1), 0)
        idx = jnp.min(jnp.where(r == rmax, tok, S - 1))
        idx = jnp.clip(idx, 0, S - 1)
        base = pl.multiple_of((idx // 16) * 16, 16)
        for c in copies[1:]:
            c.wait()
        xs = hn_ref[pl.ds(base, 16), :]
        g = _dot(xs, wg_ref[...])
        u = _dot(xs, wu_ref[...])
        act = (g * jax.nn.sigmoid(g) * u).astype(BF16)
        y = _dot(act, wd_ref[...])
        gate = jax.nn.sigmoid(jnp.full((16, 1), rmax, F32))
        row = lax.broadcasted_iota(jnp.int32, (16, 1), 0) + base
        upd = jnp.where(row == idx, y * gate, 0.0)
        out_ref[pl.ds(base, 16), :] = (out_ref[pl.ds(base, 16), :].astype(F32) + upd).astype(BF16)


@jax.jit
def pallas_sequential_preLN__mha_block__moe_arch_mod__prompt_kernel(
    A_x, A_wqkv, A_wo, B_x, B_w_r, B_w_gate, B_w_up, B_w_down,
):
    del B_x
    x = A_x.reshape(S, D)
    wr = B_w_r.reshape(1, D)
    vmem = pl.BlockSpec(memory_space=pltpu.VMEM)
    hbm = pl.BlockSpec(memory_space=pl.ANY)
    out = pl.pallas_call(
        _kernel,
        out_shape=jax.ShapeDtypeStruct((S, D), BF16),
        in_specs=[vmem, vmem, vmem, hbm, hbm, hbm, hbm],
        out_specs=vmem,
        scratch_shapes=[
            pltpu.VMEM((D, D), BF16),
            pltpu.VMEM((D, F), BF16),
            pltpu.VMEM((D, F), BF16),
            pltpu.VMEM((F, D), BF16),
            pltpu.SemaphoreType.DMA((4,)),
            pltpu.VMEM((2 * D, D), BF16),
            pltpu.VMEM((H, S, 32), BF16),
            pltpu.VMEM((NQB, D, QB), BF16),
            pltpu.VMEM((NKC, D, KC), F32),
            pltpu.VMEM((S, QB), F32),
            pltpu.VMEM((NQB, D, QB), F32),
            pltpu.VMEM((S, D), BF16),
            pltpu.VMEM((S, 1), F32),
        ],
        compiler_params=pltpu.CompilerParams(vmem_limit_bytes=100 * 2**20),
    )(x, A_wqkv, wr, A_wo, B_w_gate, B_w_up, B_w_down)
    return out.reshape(1, S, D)
```

```python
import jax
import jax.numpy as jnp
from jax import lax
from jax.experimental import pallas as pl
from jax.experimental.pallas import tpu as pltpu

S = 2048
D = 640
H = 32
DH = 20
F = 1536
QB = 512
KC = 128
NQB = S // QB
NKC = S // KC
TC = 128
SPB = 8
EPS = 1e-5
LOG2E = 1.4426950408889634
QSCALE = float(DH ** -0.5 * LOG2E)

X_SPLIT = (0, 256, 768, 1536, 2048)
O_SPLIT = (0, 1024, 1536, 1792, 2048)

VCH = (1, 3, 5, 7, 8, 10, 12, 14)
UNITS = tuple((c, half) for c in VCH for half in range(2))
UNIT_AT = tuple((i - 1,) if 0 < i < NKC - 1 else () for i in range(NKC - 1)) + ((14, 15),)
MCH = 4

BF16 = jnp.bfloat16
F32 = jnp.float32


def _dot(a, b):
    return jnp.dot(a, b, preferred_element_type=F32)


def _dot_nt(a, b):
    return lax.dot_general(a, b, (((1,), (1,)), ((), ())), preferred_element_type=F32)


def _layernorm_rows(x):
    mu = jnp.mean(x, axis=-1, keepdims=True)
    xc = x - mu
    var = jnp.mean(xc * xc, axis=-1, keepdims=True)
    return xc * lax.rsqrt(var + EPS)


def _mo(v, n):
    return v if isinstance(v, int) else pl.multiple_of(v, n)


def _pack16(v):
    return pltpu.bitcast(v, jnp.int32)


def _unpack16(v):
    return pltpu.bitcast(v, BF16)


def _kernel(x_hbm, wqkv_hbm, wr_ref, wo_hbm, wg_hbm, wu_hbm, wd_hbm,
            out_hbm,
            kp_ref, s0_ref, s1_ref, vt_ref, ot_ref, qt_ref, kf_ref, qb0_ref, qb1_ref,
            x_ref, xn_ref, kc_ref, out_ref, hn_ref,
            wq_ref, wk_ref, wv_ref, wo_ref, wqvt_ref, wg_ref, wu_ref, wd_ref,
            patch_ref,
            xsem, wsem, osem):
    def x_copy(i):
        rows = pl.ds(X_SPLIT[i], X_SPLIT[i + 1] - X_SPLIT[i])
        return pltpu.make_async_copy(x_hbm.at[rows, :], x_ref.at[rows, :], xsem.at[i])

    def out_copy(i):
        rows = pl.ds(O_SPLIT[i], O_SPLIT[i + 1] - O_SPLIT[i])
        return pltpu.make_async_copy(out_ref.at[rows, :], out_hbm.at[rows, :], osem.at[i])

    wq_c = pltpu.make_async_copy(wqkv_hbm.at[:, pl.ds(0, D)], wq_ref, wsem.at[0])
    wk_c = pltpu.make_async_copy(wqkv_hbm.at[:, pl.ds(D, D)], wk_ref, wsem.at[1])
    wv_c = pltpu.make_async_copy(wqkv_hbm.at[:, pl.ds(2 * D, D)], wv_ref, wsem.at[2])
    wo_c = pltpu.make_async_copy(wo_hbm, wo_ref, wsem.at[3])
    wg_c = pltpu.make_async_copy(wg_hbm, wg_ref, wsem.at[4])
    wu_c = pltpu.make_async_copy(wu_hbm, wu_ref, wsem.at[5])
    wd_c = pltpu.make_async_copy(wd_hbm, wd_ref, wsem.at[6])

    xn = {}

    def ln1(lo, hi):
        for c in range(lo, hi):
            v = _layernorm_rows(x_ref[pl.ds(c * TC, TC), :].astype(F32)).astype(BF16)
            xn_ref[pl.ds(c * TC // 2, TC // 2), :] = _pack16(v)
            xn[c] = v

    def kproj(lo, hi):
        for c in range(lo, hi):
            k = _dot(xn[c], wk_ref[...])
            kc_ref[pl.ds(c * TC // 2, TC // 2), :] = _pack16(k.astype(BF16))

    x_copy(0).start()
    wk_c.start()
    x_copy(0).wait()
    ln1(0, 2)
    wk_c.wait()
    x_copy(1).start()
    kproj(0, 2)
    x_copy(1).wait()
    x_copy(2).start()
    wq_c.start()
    ln1(2, 6)
    kproj(2, 6)
    x_copy(2).wait()
    x_copy(3).start()
    wv_c.start()
    ln1(6, 12)
    kproj(6, 10)
    x_copy(3).wait()
    wq_c.wait()
    wv_c.wait()
    ln1(12, 16)
    kproj(10, 16)
    wqvt_ref[0:D, :] = wq_ref[...].T
    wqvt_ref[D:2 * D, :] = wv_ref[...].T

    lane = lax.broadcasted_iota(jnp.int32, (QB // 2, 128), 1)
    for j in range(NQB):
        rows2 = pl.ds(j * (QB // 2), QB // 2)
        qv = _dot_nt(wqvt_ref[...], _unpack16(xn_ref[rows2, :]))
        qt_ref[j, :, :] = _pack16((qv[0:D, :] * QSCALE).astype(BF16))
        for u in range(QB // KC):
            vt_ref[j * (QB // KC) + u, :, :] = qv[D:2 * D, u * KC:(u + 1) * KC]
        grp = [kc_ref[rows2, pl.ds(g * 128, 128)] for g in range(D // 128)]
        for h in range(H):
            o = 16 * ((DH * h) // 16)
            lo = DH * h - o
            g, sh = o // 128, o % 128
            v = grp[g]
            if sh + lo + DH > 128:
                v = jnp.where(lane >= sh, v, grp[g + 1])
            if sh:
                v = pltpu.roll(v, 128 - sh, 1)
            kwin = jnp.where((lane >= lo) & (lane < lo + DH), v, 0)
            kp_ref[h, rows2, :] = kwin
            for i, c in enumerate(VCH):
                if c // (QB // KC) == j:
                    r = (KC // 2) * (c % (QB // KC))
                    kf_ref[h, pl.ds(16 * i, 16), :] = _unpack16(kwin[r:r + 8, :]).astype(F32)

    wo_c.start()
    wg_c.start()
    wu_c.start()
    wd_c.start()

    def chunk_rows(kc):
        return pl.ds(kc * KC, KC)

    def q_rows(blk):
        _, hb, u = blk
        return _mo((DH // 2) * hb + ((DH * u) // 16) * 8, 8)

    def v_rows(blk):
        _, hb, u = blk
        return _mo(DH * hb + ((DH * u) // 8) * 8, 8)

    def qk_mxu(blk, kc, r0=0):
        j, hb, u = blk
        k = _unpack16(kp_ref[hb + u, pl.ds(kc * (KC // 2) + r0 // 2, (KC - r0) // 2), :])[:, 0:32]
        qt = _unpack16(qt_ref[j, pl.ds(q_rows(blk), 16), :])
        return _dot(k, qt)

    def build_qb(blk, qb_ref, ds):
        j, hb, u = blk
        for d in ds:
            w = qt_ref[j, pl.ds((DH // 2) * hb + (DH // 2) * u + d // 2, 1), :]
            bits = (w << 16) if d % 2 == 0 else (w & jnp.int32(-65536))
            qb_ref[pl.ds(8 * d, 8), :] = jnp.broadcast_to(pltpu.bitcast(bits, F32), (8, QB))

    def qk_vpu(blk, unit, qb_ref):
        _, hb, u = blk
        kf = kf_ref[hb + u, pl.ds(8 * unit, 8), :]
        lo = (DH * u) % 16
        acc = None
        for d in range(DH):
            term = kf[:, lo + d:lo + d + 1] * qb_ref[pl.ds(8 * d, 8), :]
            acc = term if acc is None else acc + term
        return acc

    def finish_max(m):
        return jnp.broadcast_to(jnp.max(m, axis=0, keepdims=True), (8, QB))

    row24 = lax.broadcasted_iota(jnp.int32, (24, KC), 0)
    row8 = lax.broadcasted_iota(jnp.int32, (8, QB), 0)

    def finalize(blk, acc):
        j, hb, u = blk
        ones_row = 20 if u % 2 == 0 else 0
        ov = v_rows(blk)
        l = jnp.broadcast_to(acc[ones_row:ones_row + 1, :], (8, QB))
        r = pl.reciprocal(l, approx=True)
        inv_l = r * (2.0 - l * r)
        o0, o1, o2 = acc[0:8] * inv_l, acc[8:16] * inv_l, acc[16:24] * inv_l
        if u % 2 == 0:
            ot_ref[j, pl.ds(ov, 8), :] = o0
        else:
            first = ot_ref[j, pl.ds(ov, 8), :]
            ot_ref[j, pl.ds(ov, 8), :] = jnp.where(row8 < 4, first, o0)
        ot_ref[j, pl.ds(ov + 8, 8), :] = o1
        ot_ref[j, pl.ds(ov + 16, 8), :] = o2

    def step(blk, m_cur, nxt, nxt2, pending):
        j, hb, u = blk
        s_ref, qb_ref, qn_ref = (s0_ref, qb0_ref, qb1_ref) if u % 2 == 0 else (s1_ref, qb1_ref, qb0_ref)
        ones_row = 20 if u % 2 == 0 else 0
        ov = v_rows(blk)
        acc = jnp.zeros((24, QB), F32)
        m_prev = None
        mx = [None] * MCH

        def upd(i, v):
            mx[i] = v if mx[i] is None else jnp.maximum(mx[i], v)

        for kc in range(NKC):
            s_old = s_ref[chunk_rows(kc), :]
            r0 = 16 if kc in VCH else 0
            if nxt is not None:
                s_new = qk_mxu(nxt, kc, r0)
            p = jnp.exp2((s_old.reshape(KC // 8, 8, QB) - m_cur[None]).reshape(KC, QB)).astype(BF16)
            vt = vt_ref[kc, pl.ds(ov, 24), :]
            vt = jnp.where(row24 == ones_row, 1.0, vt)
            acc = acc + _dot(vt, p)
            if nxt is not None:
                s_ref[pl.ds(kc * KC + r0, KC - r0), :] = s_new
                upd(kc % MCH, jnp.max(s_new.reshape((KC - r0) // 8, 8, QB), axis=0))
                for un in UNIT_AT[kc]:
                    sv = qk_vpu(nxt, un, qb_ref)
                    s_ref[pl.ds(UNITS[un][0] * KC + UNITS[un][1] * 8, 8), :] = sv
                    upd(kc % MCH, sv)
            if nxt2 is not None:
                build_qb(nxt2, qn_ref, [d for d in range(DH) if 2 + d * 12 // DH == kc])
            if pending is not None and kc == 3:
                finalize(pending[0], pending[1])
            if pending is not None and kc == 5 and pending[2] is not None:
                m_prev = finish_max(pending[2])
        m_new = None
        if nxt is not None:
            for v in mx:
                m_new = v if m_new is None else jnp.maximum(m_new, v)
        return acc, m_new, m_prev

    m0 = jnp.full((8, QB), -jnp.inf, F32)
    m1 = jnp.full((8, QB), -jnp.inf, F32)
    for kc in range(NKC):
        sa = qk_mxu((0, 0, 0), kc)
        s0_ref[chunk_rows(kc), :] = sa
        m0 = jnp.maximum(m0, jnp.max(sa.reshape(KC // 8, 8, QB), axis=0))
        sb = qk_mxu((0, 0, 1), kc)
        s1_ref[chunk_rows(kc), :] = sb
        m1 = jnp.maximum(m1, jnp.max(sb.reshape(KC // 8, 8, QB), axis=0))
    m0 = finish_max(m0)
    m1 = finish_max(m1)
    build_qb((0, 0, 2), qb0_ref, range(DH))

    bpq = H // SPB
    nb = NQB * bpq

    def body(b, ms, last=False):
        j, hb = b // bpq, (b % bpq) * SPB
        if not last:
            j1, hb1 = (b + 1) // bpq, ((b + 1) % bpq) * SPB

        def blk(u):
            if u < SPB:
                return (j, hb, u)
            return None if last else (j1, hb1, u - SPB)

        ma, mb = ms
        pending = None
        for u in range(SPB):
            acc, m_raw, m_prev = step(blk(u), ma, blk(u + 2), blk(u + 3), pending)
            if pending is not None:
                mb = m_prev
            if u < SPB - 1:
                pending = (blk(u), acc, m_raw)
                ma, mb = mb, None
            else:
                finalize(blk(u), acc)
                ma, mb = mb, (finish_max(m_raw) if m_raw is not None else None)
        return ma, mb

    ms = lax.fori_loop(0, nb - 1, body, (m0, m1))
    body(nb - 1, ms, last=True)

    wo_c.wait()
    wr = wr_ref[...].astype(F32).reshape(1, D)
    tok = lax.broadcasted_iota(jnp.int32, (TC, 1), 0)
    best_v = jnp.full((1, 1), -jnp.inf, F32)
    best_i = jnp.zeros((1, 1), jnp.int32)
    for c in range(S // TC):
        rows = pl.ds(c * TC, TC)
        o = ot_ref[(c * TC) // QB, :, pl.ds((c * TC) % QB, TC)].T.astype(BF16)
        hh = x_ref[rows, :].astype(F32) + _dot(o, wo_ref[...])
        hn = _layernorm_rows(hh)
        out_ref[rows, :] = (hh + hn).astype(BF16)
        if (c + 1) * TC in O_SPLIT:
            out_copy(O_SPLIT.index((c + 1) * TC) - 1).start()
        hnb = hn.astype(BF16)
        hn_ref[pl.ds(c * TC // 2, TC // 2), :] = _pack16(hnb)
        r = jnp.sum(hnb.astype(F32) * wr, axis=-1, keepdims=True)
        cv = jnp.max(r, axis=0, keepdims=True)
        ci = jnp.min(jnp.where(r == cv, tok + c * TC, S - 1), axis=0, keepdims=True)
        take = cv > best_v
        best_v, best_i = jnp.where(take, cv, best_v), jnp.where(take, ci, best_i)

    idx = jnp.clip(jnp.max(best_i), 0, S - 1)
    base = pl.multiple_of((idx // 16) * 16, 16)
    base2 = pl.multiple_of((idx // 16) * 8, 8)
    wg_c.wait()
    wu_c.wait()
    wd_c.wait()
    xs = _unpack16(hn_ref[pl.ds(base2, 8), :])
    g = _dot(xs, wg_ref[...])
    u = _dot(xs, wu_ref[...])
    act = (g * jax.nn.sigmoid(g) * u).astype(BF16)
    y = _dot(act, wd_ref[...])
    row = lax.broadcasted_iota(jnp.int32, (16, 1), 0) + base
    upd = jnp.where(row == idx, y * jax.nn.sigmoid(best_v), 0.0)
    patch_ref[...] = (out_ref[pl.ds(base, 16), :].astype(F32) + upd).astype(BF16)
    for i in range(len(O_SPLIT) - 1):
        out_copy(i).wait()
    patch = pltpu.make_async_copy(patch_ref, out_hbm.at[pl.ds(base, 16), :], wsem.at[7])
    patch.start()
    patch.wait()


@jax.jit
def pallas_sequential_preLN__mha_block__moe_arch_mod__prompt_kernel(
    A_x: jax.Array,
    A_wqkv: jax.Array,
    A_wo: jax.Array,
    B_x: jax.Array,
    B_w_r: jax.Array,
    B_w_gate: jax.Array,
    B_w_up: jax.Array,
    B_w_down: jax.Array,
):
    del B_x
    vmem = pl.BlockSpec(memory_space=pltpu.VMEM)
    hbm = pl.BlockSpec(memory_space=pl.ANY)
    out = pl.pallas_call(
        _kernel,
        out_shape=jax.ShapeDtypeStruct((S, D), BF16),
        in_specs=[hbm, hbm, vmem, hbm, hbm, hbm, hbm],
        out_specs=hbm,
        scratch_shapes=[
            pltpu.VMEM((H, S // 2, 128), jnp.int32),
            pltpu.VMEM((S, QB), F32),
            pltpu.VMEM((S, QB), F32),
            pltpu.VMEM((NKC, D, KC), F32),
            pltpu.VMEM((NQB, D, QB), F32),
            pltpu.VMEM((NQB, D // 2, QB), jnp.int32),
            pltpu.VMEM((H, 16 * len(VCH), 128), F32),
            pltpu.VMEM((DH * 8, QB), F32),
            pltpu.VMEM((DH * 8, QB), F32),
            pltpu.VMEM((S, D), BF16),
            pltpu.VMEM((S // 2, D), jnp.int32),
            pltpu.VMEM((S // 2, D), jnp.int32),
            pltpu.VMEM((S, D), BF16),
            pltpu.VMEM((S // 2, D), jnp.int32),
            pltpu.VMEM((D, D), BF16),
            pltpu.VMEM((D, D), BF16),
            pltpu.VMEM((D, D), BF16),
            pltpu.VMEM((D, D), BF16),
            pltpu.VMEM((2 * D, D), BF16),
            pltpu.VMEM((D, F), BF16),
            pltpu.VMEM((D, F), BF16),
            pltpu.VMEM((F, D), BF16),
            pltpu.VMEM((16, D), BF16),
            pltpu.SemaphoreType.DMA((len(X_SPLIT) - 1,)),
            pltpu.SemaphoreType.DMA((8,)),
            pltpu.SemaphoreType.DMA((len(O_SPLIT) - 1,)),
        ],
        compiler_params=pltpu.CompilerParams(vmem_limit_bytes=100 * 2**20),
    )(A_x.reshape(S, D), A_wqkv, B_w_r, A_wo, B_w_gate, B_w_up, B_w_down)
    return out.reshape(1, S, D)
```

```python
import jax
import jax.numpy as jnp
from jax import lax
from jax.experimental import pallas as pl
from jax.experimental.pallas import tpu as pltpu

S = 2048
D = 640
H = 32
DH = 20
F = 1536
QB = 512
KC = 128
NQB = S // QB
NKC = S // KC
TC = 128
SPB = 8
EPS = 1e-5
LOG2E = 1.4426950408889634
QSCALE = float(DH ** -0.5 * LOG2E)

X_SPLIT = (0, 256, 768, 1536, 2048)
O_SPLIT = (0, 1024, 1536, 1792, 2048)

VCH = (1, 3, 5, 7, 8, 10, 12, 14)
UNITS = tuple((c, half) for c in VCH for half in range(2))
UNIT_AT = tuple((i - 1,) if 0 < i < NKC - 1 else () for i in range(NKC - 1)) + ((14, 15),)
MCH = 4

BF16 = jnp.bfloat16
F32 = jnp.float32


def _dot(a, b):
    return jnp.dot(a, b, preferred_element_type=F32)


def _dot_nt(a, b):
    return lax.dot_general(a, b, (((1,), (1,)), ((), ())), preferred_element_type=F32)


def _layernorm_rows(x):
    mu = jnp.mean(x, axis=-1, keepdims=True)
    xc = x - mu
    var = jnp.mean(xc * xc, axis=-1, keepdims=True)
    return xc * lax.rsqrt(var + EPS)


def _mo(v, n):
    return v if isinstance(v, int) else pl.multiple_of(v, n)


def _pack16(v):
    return pltpu.bitcast(v, jnp.int32)


def _unpack16(v):
    return pltpu.bitcast(v, BF16)


def _kernel(x_hbm, wqkv_hbm, wr_ref, wo_hbm, wg_hbm, wu_hbm, wd_hbm,
            out_hbm,
            kp_ref, s0_ref, s1_ref, vt_ref, ot_ref, qt_ref, kf_ref, qb0_ref, qb1_ref,
            x_ref, xn_ref, kc_ref, out_ref, hn_ref,
            wq_ref, wk_ref, wv_ref, wo_ref, wqvt_ref, wg_ref, wu_ref, wd_ref,
            patch_ref, wo32_ref,
            xsem, wsem, osem):
    def x_copy(i):
        rows = pl.ds(X_SPLIT[i], X_SPLIT[i + 1] - X_SPLIT[i])
        return pltpu.make_async_copy(x_hbm.at[rows, :], x_ref.at[rows, :], xsem.at[i])

    def out_copy(i):
        rows = pl.ds(O_SPLIT[i], O_SPLIT[i + 1] - O_SPLIT[i])
        return pltpu.make_async_copy(out_ref.at[rows, :], out_hbm.at[rows, :], osem.at[i])

    wq_c = pltpu.make_async_copy(wqkv_hbm.at[:, pl.ds(0, D)], wq_ref, wsem.at[0])
    wk_c = pltpu.make_async_copy(wqkv_hbm.at[:, pl.ds(D, D)], wk_ref, wsem.at[1])
    wv_c = pltpu.make_async_copy(wqkv_hbm.at[:, pl.ds(2 * D, D)], wv_ref, wsem.at[2])
    wo_c = pltpu.make_async_copy(wo_hbm, wo_ref, wsem.at[3])
    wg_c = pltpu.make_async_copy(wg_hbm, wg_ref, wsem.at[4])
    wu_c = pltpu.make_async_copy(wu_hbm, wu_ref, wsem.at[5])
    wd_c = pltpu.make_async_copy(wd_hbm, wd_ref, wsem.at[6])

    xn = {}

    def ln1(lo, hi):
        for c in range(lo, hi):
            v = _layernorm_rows(x_ref[pl.ds(c * TC, TC), :].astype(F32)).astype(BF16)
            xn_ref[pl.ds(c * TC // 2, TC // 2), :] = _pack16(v)
            xn[c] = v

    def kproj(lo, hi):
        for c in range(lo, hi):
            k = _dot(xn[c], wk_ref[...])
            kc_ref[pl.ds(c * TC // 2, TC // 2), :] = _pack16(k.astype(BF16))

    x_copy(0).start()
    wk_c.start()
    x_copy(0).wait()
    ln1(0, 2)
    wk_c.wait()
    x_copy(1).start()
    kproj(0, 2)
    x_copy(1).wait()
    x_copy(2).start()
    wq_c.start()
    ln1(2, 6)
    kproj(2, 6)
    x_copy(2).wait()
    x_copy(3).start()
    wv_c.start()
    ln1(6, 12)
    kproj(6, 10)
    x_copy(3).wait()
    wq_c.wait()
    wv_c.wait()
    ln1(12, 16)
    kproj(10, 16)
    wqvt_ref[0:D, :] = wq_ref[...].T
    wqvt_ref[D:2 * D, :] = wv_ref[...].T

    lane = lax.broadcasted_iota(jnp.int32, (QB // 2, 128), 1)
    for j in range(NQB):
        rows2 = pl.ds(j * (QB // 2), QB // 2)
        qv = _dot_nt(wqvt_ref[...], _unpack16(xn_ref[rows2, :]))
        qt_ref[j, :, :] = _pack16((qv[0:D, :] * QSCALE).astype(BF16))
        for u in range(QB // KC):
            vt_ref[j * (QB // KC) + u, :, :] = qv[D:2 * D, u * KC:(u + 1) * KC]
        grp = [kc_ref[rows2, pl.ds(g * 128, 128)] for g in range(D // 128)]
        for h in range(H):
            o = 16 * ((DH * h) // 16)
            lo = DH * h - o
            g, sh = o // 128, o % 128
            v = grp[g]
            if sh + lo + DH > 128:
                v = jnp.where(lane >= sh, v, grp[g + 1])
            if sh:
                v = pltpu.roll(v, 128 - sh, 1)
            kwin = jnp.where((lane >= lo) & (lane < lo + DH), v, 0)
            kp_ref[h, rows2, :] = kwin
            for i, c in enumerate(VCH):
                if c // (QB // KC) == j:
                    r = (KC // 2) * (c % (QB // KC))
                    kf_ref[h, pl.ds(16 * i, 16), :] = _unpack16(kwin[r:r + 8, :]).astype(F32)

    wo_c.start()
    wg_c.start()
    wu_c.start()
    wd_c.start()

    def chunk_rows(kc):
        return pl.ds(kc * KC, KC)

    def q_rows(blk):
        _, hb, u = blk
        return _mo((DH // 2) * hb + ((DH * u) // 16) * 8, 8)

    def v_rows(blk):
        _, hb, u = blk
        return _mo(DH * hb + ((DH * u) // 8) * 8, 8)

    def qk_mxu(blk, kc, r0=0):
        j, hb, u = blk
        k = _unpack16(kp_ref[hb + u, pl.ds(kc * (KC // 2) + r0 // 2, (KC - r0) // 2), :])[:, 0:32]
        qt = _unpack16(qt_ref[j, pl.ds(q_rows(blk), 16), :])
        return _dot(k, qt)

    def build_qb(blk, qb_ref, ds):
        j, hb, u = blk
        for d in ds:
            w = qt_ref[j, pl.ds((DH // 2) * hb + (DH // 2) * u + d // 2, 1), :]
            bits = (w << 16) if d % 2 == 0 else (w & jnp.int32(-65536))
            qb_ref[pl.ds(8 * d, 8), :] = jnp.broadcast_to(pltpu.bitcast(bits, F32), (8, QB))

    def qk_vpu(blk, unit, qb_ref):
        _, hb, u = blk
        kf = kf_ref[hb + u, pl.ds(8 * unit, 8), :]
        lo = (DH * u) % 16
        acc = None
        for d in range(DH):
            term = kf[:, lo + d:lo + d + 1] * qb_ref[pl.ds(8 * d, 8), :]
            acc = term if acc is None else acc + term
        return acc

    def finish_max(m):
        return jnp.broadcast_to(jnp.max(m, axis=0, keepdims=True), (8, QB))

    row24 = lax.broadcasted_iota(jnp.int32, (24, KC), 0)
    row8 = lax.broadcasted_iota(jnp.int32, (8, QB), 0)

    def finalize(blk, acc):
        j, hb, u = blk
        ones_row = 20 if u % 2 == 0 else 0
        ov = v_rows(blk)
        l = jnp.broadcast_to(acc[ones_row:ones_row + 1, :], (8, QB))
        r = pl.reciprocal(l, approx=True)
        inv_l = r * (2.0 - l * r)
        o0, o1, o2 = acc[0:8] * inv_l, acc[8:16] * inv_l, acc[16:24] * inv_l
        if u % 2 == 0:
            ot_ref[j, pl.ds(ov, 8), :] = o0
        else:
            first = ot_ref[j, pl.ds(ov, 8), :]
            ot_ref[j, pl.ds(ov, 8), :] = jnp.where(row8 < 4, first, o0)
        ot_ref[j, pl.ds(ov + 8, 8), :] = o1
        ot_ref[j, pl.ds(ov + 16, 8), :] = o2

    def step(blk, m_cur, nxt, nxt2):
        j, hb, u = blk
        s_ref, qb_ref, qn_ref = (s0_ref, qb0_ref, qb1_ref) if u % 2 == 0 else (s1_ref, qb1_ref, qb0_ref)
        ones_row = 20 if u % 2 == 0 else 0
        ov = v_rows(blk)
        acc = jnp.zeros((24, QB), F32)
        mx = [None] * MCH

        def upd(i, v):
            mx[i] = v if mx[i] is None else jnp.maximum(mx[i], v)

        for kc in range(NKC):
            s_old = s_ref[chunk_rows(kc), :]
            r0 = 16 if kc in VCH else 0
            if nxt is not None:
                s_new = qk_mxu(nxt, kc, r0)
            p = jnp.exp2((s_old.reshape(KC // 8, 8, QB) - m_cur[None]).reshape(KC, QB)).astype(BF16)
            vt = vt_ref[kc, pl.ds(ov, 24), :]
            vt = jnp.where(row24 == ones_row, 1.0, vt)
            acc = acc + _dot(vt, p)
            if nxt is not None:
                s_ref[pl.ds(kc * KC + r0, KC - r0), :] = s_new
                upd(kc % MCH, jnp.max(s_new.reshape((KC - r0) // 8, 8, QB), axis=0))
                for un in UNIT_AT[kc]:
                    sv = qk_vpu(nxt, un, qb_ref)
                    s_ref[pl.ds(UNITS[un][0] * KC + UNITS[un][1] * 8, 8), :] = sv
                    upd(kc % MCH, sv)
            if nxt2 is not None:
                build_qb(nxt2, qn_ref, [d for d in range(DH) if d * 8 // DH == kc])
        finalize(blk, acc)
        if nxt is None:
            return None
        m_new = mx[0]
        for v in mx[1:]:
            m_new = jnp.maximum(m_new, v)
        return finish_max(m_new)

    m0 = jnp.full((8, QB), -jnp.inf, F32)
    m1 = jnp.full((8, QB), -jnp.inf, F32)
    for kc in range(NKC):
        sa = qk_mxu((0, 0, 0), kc)
        s0_ref[chunk_rows(kc), :] = sa
        m0 = jnp.maximum(m0, jnp.max(sa.reshape(KC // 8, 8, QB), axis=0))
        sb = qk_mxu((0, 0, 1), kc)
        s1_ref[chunk_rows(kc), :] = sb
        m1 = jnp.maximum(m1, jnp.max(sb.reshape(KC // 8, 8, QB), axis=0))
    m0 = finish_max(m0)
    m1 = finish_max(m1)
    build_qb((0, 0, 2), qb0_ref, range(DH))

    bpq = H // SPB
    nb = NQB * bpq

    def body(b, ms, last=False):
        j, hb = b // bpq, (b % bpq) * SPB
        if not last:
            j1, hb1 = (b + 1) // bpq, ((b + 1) % bpq) * SPB

        def blk(u):
            if u < SPB:
                return (j, hb, u)
            return None if last else (j1, hb1, u - SPB)

        ma, mb = ms
        for u in range(SPB):
            ma, mb = mb, step(blk(u), ma, blk(u + 2), blk(u + 3))
        return ma, mb

    ms = lax.fori_loop(0, nb - 1, body, (m0, m1))
    body(nb - 1, ms, last=True)

    wo_c.wait()
    wo32_ref[...] = _pack16(wo_ref[...])
    wr = wr_ref[...].astype(F32).reshape(1, D)
    tok = lax.broadcasted_iota(jnp.int32, (TC, 1), 0)
    best_v = jnp.full((1, 1), -jnp.inf, F32)
    best_i = jnp.zeros((1, 1), jnp.int32)
    for c in range(S // TC):
        rows = pl.ds(c * TC, TC)
        o = ot_ref[(c * TC) // QB, :, pl.ds((c * TC) % QB, TC)].T.astype(BF16)
        hh = x_ref[rows, :].astype(F32) + _dot(o, _unpack16(wo32_ref[...]))
        hn = _layernorm_rows(hh)
        out_ref[rows, :] = (hh + hn).astype(BF16)
        if (c + 1) * TC in O_SPLIT:
            out_copy(O_SPLIT.index((c + 1) * TC) - 1).start()
        hnb = hn.astype(BF16)
        hn_ref[pl.ds(c * TC // 2, TC // 2), :] = _pack16(hnb)
        r = jnp.sum(hnb.astype(F32) * wr, axis=-1, keepdims=True)
        cv = jnp.max(r, axis=0, keepdims=True)
        ci = jnp.min(jnp.where(r == cv, tok + c * TC, S - 1), axis=0, keepdims=True)
        take = cv > best_v
        best_v, best_i = jnp.where(take, cv, best_v), jnp.where(take, ci, best_i)

    idx = jnp.clip(jnp.max(best_i), 0, S - 1)
    base = pl.multiple_of((idx // 16) * 16, 16)
    base2 = pl.multiple_of((idx // 16) * 8, 8)
    wg_c.wait()
    wu_c.wait()
    wd_c.wait()
    xs = _unpack16(hn_ref[pl.ds(base2, 8), :])
    g = _dot(xs, wg_ref[...])
    u = _dot(xs, wu_ref[...])
    act = (g * jax.nn.sigmoid(g) * u).astype(BF16)
    y = _dot(act, wd_ref[...])
    row = lax.broadcasted_iota(jnp.int32, (16, 1), 0) + base
    upd = jnp.where(row == idx, y * jax.nn.sigmoid(best_v), 0.0)
    patch_ref[...] = (out_ref[pl.ds(base, 16), :].astype(F32) + upd).astype(BF16)
    for i in range(len(O_SPLIT) - 1):
        out_copy(i).wait()
    patch = pltpu.make_async_copy(patch_ref, out_hbm.at[pl.ds(base, 16), :], wsem.at[7])
    patch.start()
    patch.wait()


@jax.jit
def pallas_sequential_preLN__mha_block__moe_arch_mod__prompt_kernel(
    A_x: jax.Array,
    A_wqkv: jax.Array,
    A_wo: jax.Array,
    B_x: jax.Array,
    B_w_r: jax.Array,
    B_w_gate: jax.Array,
    B_w_up: jax.Array,
    B_w_down: jax.Array,
):
    del B_x
    vmem = pl.BlockSpec(memory_space=pltpu.VMEM)
    hbm = pl.BlockSpec(memory_space=pl.ANY)
    out = pl.pallas_call(
        _kernel,
        out_shape=jax.ShapeDtypeStruct((S, D), BF16),
        in_specs=[hbm, hbm, vmem, hbm, hbm, hbm, hbm],
        out_specs=hbm,
        scratch_shapes=[
            pltpu.VMEM((H, S // 2, 128), jnp.int32),
            pltpu.VMEM((S, QB), F32),
            pltpu.VMEM((S, QB), F32),
            pltpu.VMEM((NKC, D, KC), F32),
            pltpu.VMEM((NQB, D, QB), F32),
            pltpu.VMEM((NQB, D // 2, QB), jnp.int32),
            pltpu.VMEM((H, 16 * len(VCH), 128), F32),
            pltpu.VMEM((DH * 8, QB), F32),
            pltpu.VMEM((DH * 8, QB), F32),
            pltpu.VMEM((S, D), BF16),
            pltpu.VMEM((S // 2, D), jnp.int32),
            pltpu.VMEM((S // 2, D), jnp.int32),
            pltpu.VMEM((S, D), BF16),
            pltpu.VMEM((S // 2, D), jnp.int32),
            pltpu.VMEM((D, D), BF16),
            pltpu.VMEM((D, D), BF16),
            pltpu.VMEM((D, D), BF16),
            pltpu.VMEM((D, D), BF16),
            pltpu.VMEM((2 * D, D), BF16),
            pltpu.VMEM((D, F), BF16),
            pltpu.VMEM((D, F), BF16),
            pltpu.VMEM((F, D), BF16),
            pltpu.VMEM((16, D), BF16),
            pltpu.VMEM((D // 2, D), jnp.int32),
            pltpu.SemaphoreType.DMA((len(X_SPLIT) - 1,)),
            pltpu.SemaphoreType.DMA((8,)),
            pltpu.SemaphoreType.DMA((len(O_SPLIT) - 1,)),
        ],
        compiler_params=pltpu.CompilerParams(vmem_limit_bytes=100 * 2**20),
    )(A_x.reshape(S, D), A_wqkv, B_w_r, A_wo, B_w_gate, B_w_up, B_w_down)
    return out.reshape(1, S, D)
```
